```python
import jax
import jax.numpy as jnp

def _softmax(x, axis=-1):
    return jax.nn.softmax(x, axis=axis)

def _gelu(x):
    return jax.nn.gelu(x, approximate=True)

def _silu(x):
    return jax.nn.silu(x)

def _sigmoid(x):
    return jax.nn.sigmoid(x)

def _layernorm(x, axis=-1, eps=1e-05):
    m = jnp.mean(x, axis=axis, keepdims=True)
    v = jnp.var(x, axis=axis, keepdims=True)
    return (x - m) / jnp.sqrt(v + eps)

def _scatter_add(tgt, idx, src, axis=0):
    return tgt.at[idx].add(src)

def _segment_sum(src, seg, n):
    return jax.ops.segment_sum(src, seg, n)

class _Rng:

    def __init__(self, key):
        self._k = key

    def _next(self):
        self._k, sub = jax.random.split(self._k)
        return sub

    def normal(self, shape):
        return jax.random.normal(self._next(), shape, dtype=jnp.bfloat16)

    def randint(self, lo, hi, shape):
        return jax.random.randint(self._next(), shape, lo, hi, dtype=jnp.int32)

    def uniform(self, shape, lo=0.0, hi=1.0):
        return jax.random.uniform(self._next(), shape, jnp.bfloat16, lo, hi)

    def permutation(self, n):
        return jax.random.permutation(self._next(), n)
kernel_name = 'adaLN_cond__ssm_conv_h3__mixer_s_mlp__prompt'

def setup_inputs():
    _rng = _Rng(jax.random.key(int.from_bytes(__import__("os").urandom(4), "little")))
    _w = lambda a: (lambda t: t.astype(jnp.bfloat16) if jnp.issubdtype(t.dtype, jnp.floating) else t)(jnp.asarray(a))

    def _A_setup():
        B, S, D = (1, 2048, 640)
        ks = 4
        return {'q': _w((lambda *s: _rng.normal(s) * 0.05)(B, S, D)), 'k': _w((lambda *s: _rng.normal(s) * 0.05)(B, S, D)), 'v': _w((lambda *s: _rng.normal(s) * 0.05)(B, S, D)), 'shift_k': _w((lambda *s: _rng.normal(s) * 0.05)(D, ks) * 0.5), 'ssm_k': _w((lambda *s: _rng.normal(s) * 0.05)(D, S) * (1.0 / S ** 0.5)), 'ssm_D': _w((lambda *s: _rng.normal(s) * 0.05)(D))}
    _A_in = _A_setup()

    def _B_setup():
        B, S, D, F = (1, 2048, 640, 1728)
        return {'x': _w((lambda *s: _rng.normal(s) * 0.05)(B, S, D)), 'w1': _w((lambda *s: _rng.normal(s) * 0.05)(D, D) * D ** (-0.5)), 'w2': _w((lambda *s: _rng.normal(s) * 0.05)(D, D) * D ** (-0.5)), 'w3': _w((lambda *s: _rng.normal(s) * 0.05)(D, F) * D ** (-0.5)), 'w4': _w((lambda *s: _rng.normal(s) * 0.05)(F, D) * F ** (-0.5))}
    _B_in = _B_setup()
    return {'A_q': _A_in['q'], 'A_k': _A_in['k'], 'A_v': _A_in['v'], 'A_shift_k': _A_in['shift_k'], 'A_ssm_k': _A_in['ssm_k'], 'A_ssm_D': _A_in['ssm_D'], 'B_x': _B_in['x'], 'B_w1': _B_in['w1'], 'B_w2': _B_in['w2'], 'B_w3': _B_in['w3'], 'B_w4': _B_in['w4'], 'c': _w((lambda *s: _rng.normal(s) * 0.05)(1, 640)), 'w_mod': _w((lambda *s: _rng.normal(s) * 0.05)(640, 6 * 640) * 640 ** (-0.5))}

def reference(A_q, A_k, A_v, A_shift_k, A_ssm_k, A_ssm_D, B_x, B_w1, B_w2, B_w3, B_w4, c, w_mod):

    def _A_ref(q, k, v, shift_k, ssm_k, ssm_D):
        B, S, D = q.shape
        ks = shift_k.shape[-1]
        k_pad = jnp.pad(k, ((0, 0), (ks - 1, 0), (0, 0)))
        k_shift = jnp.zeros_like(k)
        for t in range(ks):
            k_shift = k_shift + k_pad[:, t:t + S, :] * shift_k[:, ks - 1 - t][None, None, :]
        kv = k_shift * v
        L = 2 * S
        kv_pad = jnp.pad(kv, ((0, 0), (0, S), (0, 0)))
        kf_pad = jnp.pad(ssm_k, ((0, 0), (0, S)))
        kv_f = (lambda x, axes=(-2, -1): jnp.fft.rfft2(x.astype(jnp.float32), axes=axes))(kv_pad[:, None, :, :], axes=(1, 2))
        kf_f = (lambda x, axes=(-2, -1): jnp.fft.rfft2(x.astype(jnp.float32), axes=axes))(kf_pad[:, None, :], axes=(1, 2))
        kf_f = (lambda x, *d: x.transpose(*d))(kf_f, 1, 2, 0)
        y_f = kv_f * kf_f[None, :, :, :]
        y = (lambda x, s, axes=(-2, -1): jnp.fft.irfft2(x, s=s, axes=axes).astype(jnp.bfloat16))(y_f, (1, L), axes=(1, 2))[:, 0, :S, :]
        y = y + kv * ssm_D[None, None, :]
        return q * y

    def _B_ref(x, w1, w2, w3, w4):
        B, S, D = x.shape
        h = _gelu(_layernorm(x, axis=-1) @ w1)
        c = D // 4
        g0 = jnp.pad(h[:, :, 0 * c:1 * c], ((0, 0), (1, 0), (0, 0)))[:, :S, :]
        g1 = jnp.pad(h[:, :, 1 * c:2 * c], ((0, 0), (0, 1), (0, 0)))[:, 1:, :]
        g2 = jnp.pad(h[:, :, 2 * c:3 * c], ((0, 0), (2, 0), (0, 0)))[:, :S, :]
        g3 = jnp.pad(h[:, :, 3 * c:], ((0, 0), (0, 2), (0, 0)))[:, 2:, :]
        hs = jnp.concatenate([g0, g1, g2, g3], axis=-1) @ w2
        x1 = x + hs
        h2 = _gelu(_layernorm(x1, axis=-1) @ w3) @ w4
        return x1 + h2
    x = A_q
    mod = (_silu(c) @ w_mod).reshape(c.shape[0], 6, 1, -1)
    sa, ca, ga, sb, cb, gb = (mod[:, 0].copy(), mod[:, 1].copy(), mod[:, 2].copy(), mod[:, 3].copy(), mod[:, 4].copy(), mod[:, 5].copy())
    h = _layernorm(x, axis=-1) * (1 + ca) + sa
    x = x + ga * _A_ref(h, A_k, A_v, A_shift_k, A_ssm_k, A_ssm_D)
    h = _layernorm(x, axis=-1) * (1 + cb) + sb
    x = x + gb * _B_ref(h, B_w1, B_w2, B_w3, B_w4)
    return x
```

```python
import jax
import jax.numpy as jnp
import numpy as np
import jax.experimental.pallas as pl
import jax.experimental.pallas.tpu as pltpu

S, D, F = 2048, 640, 1728
C = 128
P = S // C
CB = 128
NC = D // CB
T = 256
NB = S // T
PAD = 8
BF, F32 = jnp.bfloat16, jnp.float32


def _dft_mats():
    k = np.arange(C)[:, None]
    n = np.arange(C)[None, :]
    ang = np.pi * (2 * k + 1) * n / (2 * C)
    fwd = np.concatenate([np.cos(ang), -np.sin(ang)], 0)
    inv = np.concatenate([np.cos(ang).T, -np.sin(ang).T], 1) / C
    return fwd.astype(BF), inv.astype(BF)


def _ln(x):
    m = jnp.mean(x, axis=-1, keepdims=True)
    xc = x - m
    v = jnp.mean(xc * xc, axis=-1, keepdims=True)
    return xc * jax.lax.rsqrt(v + 1e-5)


def _gelu(x):
    u = x * (0.7978845608028654 + (0.7978845608028654 * 0.044715) * (x * x))
    hx = 0.5 * x
    return hx + hx * jnp.tanh(u)


def _dot(a, b):
    return jnp.dot(a, b, preferred_element_type=F32)


def _dot_t(a, b):
    return jax.lax.dot_general(a, b, (((1,), (1,)), ((), ())), preferred_element_type=F32)


def _kernel(k_ref, v_ref, sk_ref, f_ref, sd_ref, fwd_ref, inv_ref, q_ref, c_ref,
            wm_h, w1_h, w2_h, w3_h, w4_h, o_ref,
            wm, w1, w2, w3, w4, sems, kp, kv_s, xs, hs, ys, y_s, mod, x_s, h_s, h1_s):
    step = pl.program_id(0)
    copies = [pltpu.make_async_copy(a, b, sems.at[i]) for i, (a, b) in
              enumerate([(wm_h, wm), (w1_h, w1), (w2_h, w2), (w3_h, w3), (w4_h, w4)])]

    @pl.when(step == 0)
    def _():
        for cp in copies:
            cp.start()
        kp[0:PAD, :] = jnp.zeros((PAD, CB), F32)
        h1_s[0:PAD, :] = jnp.zeros((PAD, D), F32)
        h1_s[PAD + S:, :] = jnp.zeros((PAD, D), F32)

    @pl.when(step < NC)
    def _conv():
        skt = sk_ref[...].astype(F32)
        kp[PAD:, :] = k_ref[...].astype(F32)
        fwd = fwd_ref[...]
        par = jax.lax.broadcasted_iota(jnp.int32, (C, CB), 0) & 1
        sgn = (1 - 2 * par).astype(F32)
        prev = None
        for p in range(P):
            r = PAD + p * C
            ks = kp[r:r + C, :] * skt[0:1]
            for j in range(1, 4):
                ks = ks + kp[r - j:r - j + C, :] * skt[j:j + 1]
            kv = ks * v_ref[p * C:(p + 1) * C, :].astype(F32)
            kv_s[p * C:(p + 1) * C, :] = kv
            x = _dot(fwd, kv.astype(BF))
            xr, xi = x[:C], x[C:]
            a, b = xr, xi
            if prev is not None:
                a = xr - sgn * prev[1]
                b = xi + sgn * prev[0]
            prev = (xr, xi)
            xs[0, p], xs[1, p], xs[2, p] = a + b, a, b
            h = _dot_t(fwd, f_ref[:, p * C:(p + 1) * C])
            hr, hi = h[:C], h[C:]
            hs[0, p], hs[1, p], hs[2, p] = hr, hi - hr, hr + hi

        def mac(g, _):
            rows = pl.ds(pl.multiple_of(g * 16, 16), 16)

            def cconv(t):
                A = [xs[t, j, rows, :] for j in range(P)]
                B = [hs[t, j, rows, :] for j in range(P)]
                out = []
                for i in range(P):
                    acc = A[0] * B[i]
                    for j in range(1, i + 1):
                        acc = acc + A[j] * B[i - j]
                    out.append(acc)
                return out
            k1 = cconv(0)
            k3 = cconv(2)
            for i in range(P):
                ys[i, 0, rows, :] = (k1[i] - k3[i]).astype(BF)
            k2 = cconv(1)
            for i in range(P):
                ys[i, 1, rows, :] = (k1[i] + k2[i]).astype(BF)
            return 0
        jax.lax.fori_loop(0, C // 16, mac, 0)

        inv = inv_ref[...]
        sd = sd_ref[...].astype(F32)
        for p in range(P):
            y = _dot(inv, ys[p].reshape(2 * C, CB))
            y_s[step, p * C:(p + 1) * C, :] = y + kv_s[p * C:(p + 1) * C, :] * sd

    @pl.when(step == NC)
    def _():
        for cp in copies:
            cp.wait()
        cf = c_ref[...].astype(F32)
        sc = jnp.broadcast_to(cf * jax.nn.sigmoid(cf), (8, D)).astype(BF)
        mod[...] = _dot(sc, wm[...])

    @pl.when(step > NC)
    def _stage2():
        r0 = pl.multiple_of((step - NC - 1) * T, T)
        lane = jax.lax.broadcasted_iota(jnp.int32, (T, 128), 1)

        def ld(off, t):
            win = h1_s[pl.ds(r0, T + 2 * PAD), t * 128:(t + 1) * 128]
            return win[PAD + off:PAD + off + T, :]
        g = jnp.concatenate([
            ld(-1, 0),
            jnp.where(lane < 32, ld(-1, 1), ld(1, 1)),
            jnp.where(lane < 64, ld(1, 2), ld(-2, 2)),
            jnp.where(lane < 96, ld(-2, 3), ld(2, 3)),
            ld(2, 4)], axis=1).astype(BF)
        x1 = h_s[pl.ds(r0, T), :] + _dot(g, w2[...])
        u = _gelu(_dot_t(_ln(x1).astype(BF), w3[...])).astype(BF)
        r = x1 + _dot(u, w4[...])
        o_ref[...] = (x_s[pl.ds(r0, T), :] + mod[0:1, 5 * D:] * r).astype(BF)

    @pl.when(jnp.logical_and(step >= NC, step < NC + NB))
    def _stage1():
        r0 = pl.multiple_of((step - NC) * T, T)
        m = lambda i: mod[0:1, i * D:(i + 1) * D]
        q = q_ref[...].astype(F32)
        y = jnp.concatenate([y_s[j, pl.ds(r0, T), :] for j in range(NC)], axis=1)
        x = q + m(2) * ((_ln(q) * (1 + m(1)) + m(0)) * y)
        x_s[pl.ds(r0, T), :] = x
        h = _ln(x) * (1 + m(4)) + m(3)
        h_s[pl.ds(r0, T), :] = h
        h1_s[pl.ds(r0 + PAD, T), :] = _gelu(_dot(_ln(h).astype(BF), w1[...]))


@jax.jit
def pallas_adaLN_cond__ssm_conv_h3__mixer_s_mlp__prompt_kernel(
        A_q, A_k, A_v, A_shift_k, A_ssm_k, A_ssm_D, B_x, B_w1, B_w2, B_w3, B_w4, c, w_mod):
    fwd, inv = _dft_mats()
    cb = lambda s: jnp.minimum(s, NC - 1)
    full = lambda shp: pl.BlockSpec(shp, lambda s: (0, 0))
    hbm = pl.BlockSpec(memory_space=pl.ANY)
    vm = pltpu.VMEM
    out = pl.pallas_call(
        _kernel,
        grid=(NC + NB + 1,),
        in_specs=[
            pl.BlockSpec((S, CB), lambda s: (0, cb(s))),
            pl.BlockSpec((S, CB), lambda s: (0, cb(s))),
            pl.BlockSpec((4, CB), lambda s: (0, cb(s))),
            pl.BlockSpec((CB, S), lambda s: (cb(s), 0)),
            pl.BlockSpec((1, CB), lambda s: (0, cb(s))),
            full((2 * C, C)), full((C, 2 * C)),
            pl.BlockSpec((T, D), lambda s: (jnp.clip(s - NC, 0, NB - 1), 0)),
            full((1, D)), hbm, hbm, hbm, hbm, hbm,
        ],
        out_specs=pl.BlockSpec((T, D), lambda s: (jnp.clip(s - NC - 1, 0, NB - 1), 0)),
        out_shape=jax.ShapeDtypeStruct((S, D), BF),
        scratch_shapes=[
            vm((D, 6 * D), BF), vm((D, D), BF), vm((D, D), BF), vm((F, D), BF), vm((F, D), BF),
            pltpu.SemaphoreType.DMA((5,)),
            vm((S + PAD, CB), F32), vm((S, CB), F32),
            vm((3, P, C, CB), F32), vm((3, P, C, CB), F32), vm((P, 2, C, CB), BF),
            vm((NC, S, CB), F32), vm((8, 6 * D), F32),
            vm((S, D), F32), vm((S, D), F32), vm((S + 2 * PAD, D), F32),
        ],
        compiler_params=pltpu.CompilerParams(
            dimension_semantics=("arbitrary",), vmem_limit_bytes=100 * 1024 * 1024),
    )(A_k.reshape(S, D), A_v.reshape(S, D), A_shift_k.T, A_ssm_k, A_ssm_D.reshape(1, D),
      jnp.asarray(fwd), jnp.asarray(inv), A_q.reshape(S, D), c, w_mod, B_w1, B_w2, B_w3.T, B_w4)
    return out.reshape(1, S, D)
```

```python
import jax
import jax.numpy as jnp
import numpy as np
import jax.experimental.pallas as pl
import jax.experimental.pallas.tpu as pltpu

S, D, F = 2048, 640, 1728
C = 128
P = S // C
CB = 128
NC = D // CB
T = 512
NB = S // T
PAD = 8
BF, F32 = jnp.bfloat16, jnp.float32


def _dft_mats():
    k = np.arange(C)[:, None]
    n = np.arange(C)[None, :]
    ang = np.pi * (2 * k + 1) * n / (2 * C)
    fwd = np.concatenate([np.cos(ang), -np.sin(ang)], 0)
    inv = np.concatenate([np.cos(ang).T, -np.sin(ang).T], 1) / C
    return fwd.astype(BF), inv.astype(BF)


def _ln(x):
    m = jnp.mean(x, axis=-1, keepdims=True)
    xc = x - m
    v = jnp.mean(xc * xc, axis=-1, keepdims=True)
    return xc * jax.lax.rsqrt(v + 1e-5)


def _gelu(x):
    u = x * (0.7978845608028654 + (0.7978845608028654 * 0.044715) * (x * x))
    hx = 0.5 * x
    return hx + hx * jnp.tanh(u)


def _dot(a, b):
    return jnp.dot(a, b, preferred_element_type=F32)


def _dot_t(a, b):
    return jax.lax.dot_general(a, b, (((1,), (1,)), ((), ())), preferred_element_type=F32)


def _kernel(k_ref, v_ref, sk_ref, f_ref, sd_ref, fwd_ref, inv_ref, q_ref, c_ref,
            wm_h, w1_h, w2_h, w3_h, w4_h, o_ref,
            wm, w1, w2, w3, w4, sems, kp, kv_s, xs, hs, ys, y_s, mod, x_s, h_s, h1_s):
    step = pl.program_id(0)
    copies = [pltpu.make_async_copy(a, b, sems.at[i]) for i, (a, b) in
              enumerate([(wm_h, wm), (w1_h, w1), (w2_h, w2), (w3_h, w3), (w4_h, w4)])]

    @pl.when(step == 0)
    def _():
        for cp in copies:
            cp.start()
        kp[0:PAD, :] = jnp.zeros((PAD, CB), F32)
        h1_s[0:PAD, :] = jnp.zeros((PAD, D), F32)
        h1_s[PAD + S:, :] = jnp.zeros((PAD, D), F32)

    @pl.when(step < NC)
    def _conv():
        skt = sk_ref[...].astype(F32)
        kp[PAD:, :] = k_ref[...].astype(F32)
        fwd = fwd_ref[...]
        par = jax.lax.broadcasted_iota(jnp.int32, (C, CB), 0) & 1
        sgn = (1 - 2 * par).astype(F32)
        prev = None
        for p in range(P):
            r = PAD + p * C
            ks = kp[r:r + C, :] * skt[0:1]
            for j in range(1, 4):
                ks = ks + kp[r - j:r - j + C, :] * skt[j:j + 1]
            kv = ks * v_ref[p * C:(p + 1) * C, :].astype(F32)
            kv_s[p * C:(p + 1) * C, :] = kv
            x = _dot(fwd, kv.astype(BF))
            xr, xi = x[:C], x[C:]
            a, b = xr, xi
            if prev is not None:
                a = xr - sgn * prev[1]
                b = xi + sgn * prev[0]
            prev = (xr, xi)
            xs[0, p], xs[1, p], xs[2, p] = a + b, a, b
            h = _dot_t(fwd, f_ref[:, p * C:(p + 1) * C])
            hr, hi = h[:C], h[C:]
            hs[0, p], hs[1, p], hs[2, p] = hr, hi - hr, hr + hi

        def mac(g, _):
            rows = pl.ds(pl.multiple_of(g * 16, 16), 16)

            def cconv(t):
                A = [xs[t, j, rows, :] for j in range(P)]
                B = [hs[t, j, rows, :] for j in range(P)]
                out = []
                for i in range(P):
                    acc = A[0] * B[i]
                    for j in range(1, i + 1):
                        acc = acc + A[j] * B[i - j]
                    out.append(acc)
                return out
            k1 = cconv(0)
            k3 = cconv(2)
            for i in range(P):
                ys[i, 0, rows, :] = (k1[i] - k3[i]).astype(BF)
            k2 = cconv(1)
            for i in range(P):
                ys[i, 1, rows, :] = (k1[i] + k2[i]).astype(BF)
            return 0
        jax.lax.fori_loop(0, C // 16, mac, 0)

        inv = inv_ref[...]
        sd = sd_ref[...].astype(F32)
        for p in range(P):
            y = _dot(inv, ys[p].reshape(2 * C, CB))
            y_s[step, p * C:(p + 1) * C, :] = y + kv_s[p * C:(p + 1) * C, :] * sd

    @pl.when(step == NC)
    def _():
        for cp in copies:
            cp.wait()
        cf = c_ref[...].astype(F32)
        sc = jnp.broadcast_to(cf * jax.nn.sigmoid(cf), (8, D)).astype(BF)
        mod[...] = _dot(sc, wm[...])

    def _stage2():
        r0 = pl.multiple_of((step - NC - 1) * T, T)
        lane = jax.lax.broadcasted_iota(jnp.int32, (T, 128), 1)

        def ld(off, t):
            win = h1_s[pl.ds(r0, T + 2 * PAD), t * 128:(t + 1) * 128]
            return win[PAD + off:PAD + off + T, :]
        g = jnp.concatenate([
            ld(-1, 0),
            jnp.where(lane < 32, ld(-1, 1), ld(1, 1)),
            jnp.where(lane < 64, ld(1, 2), ld(-2, 2)),
            jnp.where(lane < 96, ld(-2, 3), ld(2, 3)),
            ld(2, 4)], axis=1).astype(BF)
        x1 = h_s[pl.ds(r0, T), :] + _dot(g, w2[...])
        u = _gelu(_dot_t(_ln(x1).astype(BF), w3[...])).astype(BF)
        r = x1 + _dot(u, w4[...])
        o_ref[...] = (x_s[pl.ds(r0, T), :] + mod[0:1, 5 * D:] * r).astype(BF)

    def _stage1():
        r0 = pl.multiple_of((step - NC) * T, T)
        m = lambda i: mod[0:1, i * D:(i + 1) * D]
        q = q_ref[...].astype(F32)
        y = jnp.concatenate([y_s[j, pl.ds(r0, T), :] for j in range(NC)], axis=1)
        x = q + m(2) * ((_ln(q) * (1 + m(1)) + m(0)) * y)
        x_s[pl.ds(r0, T), :] = x
        h = _ln(x) * (1 + m(4)) + m(3)
        h_s[pl.ds(r0, T), :] = h
        h1_s[pl.ds(r0 + PAD, T), :] = _gelu(_dot(_ln(h).astype(BF), w1[...]))

    pl.when(step == NC)(_stage1)

    @pl.when(jnp.logical_and(step > NC, step < NC + NB))
    def _():
        _stage2()
        _stage1()

    pl.when(step == NC + NB)(_stage2)


@jax.jit
def pallas_adaLN_cond__ssm_conv_h3__mixer_s_mlp__prompt_kernel(
        A_q, A_k, A_v, A_shift_k, A_ssm_k, A_ssm_D, B_x, B_w1, B_w2, B_w3, B_w4, c, w_mod):
    fwd, inv = _dft_mats()
    cb = lambda s: jnp.minimum(s, NC - 1)
    full = lambda shp: pl.BlockSpec(shp, lambda s: (0, 0))
    hbm = pl.BlockSpec(memory_space=pl.ANY)
    vm = pltpu.VMEM
    out = pl.pallas_call(
        _kernel,
        grid=(NC + NB + 1,),
        in_specs=[
            pl.BlockSpec((S, CB), lambda s: (0, cb(s))),
            pl.BlockSpec((S, CB), lambda s: (0, cb(s))),
            pl.BlockSpec((4, CB), lambda s: (0, cb(s))),
            pl.BlockSpec((CB, S), lambda s: (cb(s), 0)),
            pl.BlockSpec((1, CB), lambda s: (0, cb(s))),
            full((2 * C, C)), full((C, 2 * C)),
            pl.BlockSpec((T, D), lambda s: (jnp.clip(s - NC, 0, NB - 1), 0)),
            full((1, D)), hbm, hbm, hbm, hbm, hbm,
        ],
        out_specs=pl.BlockSpec((T, D), lambda s: (jnp.clip(s - NC - 1, 0, NB - 1), 0)),
        out_shape=jax.ShapeDtypeStruct((S, D), BF),
        scratch_shapes=[
            vm((D, 6 * D), BF), vm((D, D), BF), vm((D, D), BF), vm((F, D), BF), vm((F, D), BF),
            pltpu.SemaphoreType.DMA((5,)),
            vm((S + PAD, CB), F32), vm((S, CB), F32),
            vm((3, P, C, CB), F32), vm((3, P, C, CB), F32), vm((P, 2, C, CB), BF),
            vm((NC, S, CB), F32), vm((8, 6 * D), F32),
            vm((S, D), F32), vm((S, D), F32), vm((S + 2 * PAD, D), F32),
        ],
        compiler_params=pltpu.CompilerParams(
            dimension_semantics=("arbitrary",), vmem_limit_bytes=100 * 1024 * 1024),
    )(A_k.reshape(S, D), A_v.reshape(S, D), A_shift_k.T, A_ssm_k, A_ssm_D.reshape(1, D),
      jnp.asarray(fwd), jnp.asarray(inv), A_q.reshape(S, D), c, w_mod, B_w1, B_w2, B_w3.T, B_w4)
    return out.reshape(1, S, D)
```

```python
import jax
import jax.numpy as jnp
import numpy as np
import jax.experimental.pallas as pl
import jax.experimental.pallas.tpu as pltpu

S, D, F = 2048, 640, 1728
C = 128
P = S // C
CB = 128
NC = D // CB
T = 512
NB = S // T
PAD = 8
BF, F32 = jnp.bfloat16, jnp.float32


def _dft_mats():
    k = np.arange(C)[:, None]
    n = np.arange(C)[None, :]
    ang = np.pi * (2 * k + 1) * n / (2 * C)
    fwd = np.concatenate([np.cos(ang), -np.sin(ang)], 0)
    inv = np.concatenate([np.cos(ang).T, -np.sin(ang).T], 1) / C
    return fwd.astype(BF), inv.astype(BF)


def _ln(x):
    m = jnp.mean(x, axis=-1, keepdims=True)
    xc = x - m
    v = jnp.mean(xc * xc, axis=-1, keepdims=True)
    return xc * jax.lax.rsqrt(v + 1e-5)


def _gelu(x):
    u = x * (0.7978845608028654 + (0.7978845608028654 * 0.044715) * (x * x))
    hx = 0.5 * x
    return hx + hx * jnp.tanh(u)


def _dot(a, b):
    return jnp.dot(a, b, preferred_element_type=F32)


def _dot_t(a, b):
    return jax.lax.dot_general(a, b, (((1,), (1,)), ((), ())), preferred_element_type=F32)


def _kernel(k_ref, v_ref, sk_ref, f_ref, sd_ref, fwd_ref, inv_ref, q_ref, c_ref,
            wm_h, w1_h, w2_h, w3_h, w4_h, o_ref,
            wm, w1, w2, w3, w4, sems, kp, kv_s, xs, hs, ys, y_s, mod, x_s, h_s, h1_s):
    step = pl.program_id(0)
    copies = [pltpu.make_async_copy(a, b, sems.at[i]) for i, (a, b) in
              enumerate([(wm_h, wm), (w1_h, w1), (w2_h, w2), (w3_h, w3), (w4_h, w4)])]

    @pl.when(step == 0)
    def _():
        for cp in copies:
            cp.start()
        kp[0:PAD, :] = jnp.zeros((PAD, CB), F32)
        h1_s[0:PAD, :] = jnp.zeros((PAD, D), F32)
        h1_s[PAD + S:, :] = jnp.zeros((PAD, D), F32)

    @pl.when(step < NC)
    def _conv():
        skt = sk_ref[...].astype(F32)
        kp[PAD:, :] = k_ref[...].astype(F32)
        fwd = fwd_ref[...]
        par = jax.lax.broadcasted_iota(jnp.int32, (C, CB), 0) & 1
        sgn = (1 - 2 * par).astype(F32)
        prev = None
        for p in range(P):
            r = PAD + p * C
            ks = kp[r:r + C, :] * skt[0:1]
            for j in range(1, 4):
                ks = ks + kp[r - j:r - j + C, :] * skt[j:j + 1]
            kv = ks * v_ref[p * C:(p + 1) * C, :].astype(F32)
            kv_s[p * C:(p + 1) * C, :] = kv
            x = _dot(fwd, kv.astype(BF))
            xr, xi = x[:C], x[C:]
            a, b = xr, xi
            if prev is not None:
                a = xr - sgn * prev[1]
                b = xi + sgn * prev[0]
            prev = (xr, xi)
            xs[0, p], xs[1, p], xs[2, p] = a + b, a, b
            h = _dot_t(fwd, f_ref[:, p * C:(p + 1) * C])
            hr, hi = h[:C], h[C:]
            hs[0, p], hs[1, p], hs[2, p] = hr, hi - hr, hr + hi

        def mac(g, _):
            rows = pl.ds(pl.multiple_of(g * 16, 16), 16)

            def cconv(t):
                A = [xs[t, j, rows, :] for j in range(P)]
                B = [hs[t, j, rows, :] for j in range(P)]
                out = []
                for i in range(P):
                    acc = A[0] * B[i]
                    for j in range(1, i + 1):
                        acc = acc + A[j] * B[i - j]
                    out.append(acc)
                return out
            k1 = cconv(0)
            k3 = cconv(2)
            for i in range(P):
                ys[i, 0, rows, :] = (k1[i] - k3[i]).astype(BF)
            k2 = cconv(1)
            for i in range(P):
                ys[i, 1, rows, :] = (k1[i] + k2[i]).astype(BF)
            return 0
        jax.lax.fori_loop(0, C // 16, mac, 0)

        inv = inv_ref[...]
        sd = sd_ref[...].astype(F32)
        for p in range(P):
            y = _dot(inv, ys[p].reshape(2 * C, CB))
            y_s[step, p * C:(p + 1) * C, :] = y + kv_s[p * C:(p + 1) * C, :] * sd

    @pl.when(step == NC)
    def _():
        for cp in copies:
            cp.wait()
        cf = c_ref[...].astype(F32)
        sc = jnp.broadcast_to(cf * jax.nn.sigmoid(cf), (8, D)).astype(BF)
        mod[...] = _dot(sc, wm[...])

    def _stage2():
        r0 = pl.multiple_of((step - NC - 2) * T, T)
        lane = jax.lax.broadcasted_iota(jnp.int32, (T, 128), 1)

        def ld(off, t):
            win = h1_s[pl.ds(r0, T + 2 * PAD), t * 128:(t + 1) * 128]
            return win[PAD + off:PAD + off + T, :]
        g = jnp.concatenate([
            ld(-1, 0),
            jnp.where(lane < 32, ld(-1, 1), ld(1, 1)),
            jnp.where(lane < 64, ld(1, 2), ld(-2, 2)),
            jnp.where(lane < 96, ld(-2, 3), ld(2, 3)),
            ld(2, 4)], axis=1).astype(BF)
        x1 = h_s[pl.ds(r0, T), :] + _dot(g, w2[...])
        u = _gelu(_dot_t(_ln(x1).astype(BF), w3[...])).astype(BF)
        r = x1 + _dot(u, w4[...])
        o_ref[...] = (x_s[pl.ds(r0, T), :] + mod[0:1, 5 * D:] * r).astype(BF)

    def _stage1():
        r0 = pl.multiple_of((step - NC) * T, T)
        m = lambda i: mod[0:1, i * D:(i + 1) * D]
        q = q_ref[...].astype(F32)
        y = jnp.concatenate([y_s[j, pl.ds(r0, T), :] for j in range(NC)], axis=1)
        x = q + m(2) * ((_ln(q) * (1 + m(1)) + m(0)) * y)
        x_s[pl.ds(r0, T), :] = x
        h = _ln(x) * (1 + m(4)) + m(3)
        h_s[pl.ds(r0, T), :] = h
        h1_s[pl.ds(r0 + PAD, T), :] = _gelu(_dot(_ln(h).astype(BF), w1[...]))

    pl.when(jnp.logical_and(step >= NC, step < NC + 2))(_stage1)

    @pl.when(jnp.logical_and(step >= NC + 2, step < NC + NB))
    def _():
        _stage2()
        _stage1()

    pl.when(step >= NC + NB)(_stage2)


@jax.jit
def pallas_adaLN_cond__ssm_conv_h3__mixer_s_mlp__prompt_kernel(
        A_q, A_k, A_v, A_shift_k, A_ssm_k, A_ssm_D, B_x, B_w1, B_w2, B_w3, B_w4, c, w_mod):
    fwd, inv = _dft_mats()
    cb = lambda s: jnp.minimum(s, NC - 1)
    full = lambda shp: pl.BlockSpec(shp, lambda s: (0, 0))
    hbm = pl.BlockSpec(memory_space=pl.ANY)
    vm = pltpu.VMEM
    out = pl.pallas_call(
        _kernel,
        grid=(NC + NB + 2,),
        in_specs=[
            pl.BlockSpec((S, CB), lambda s: (0, cb(s))),
            pl.BlockSpec((S, CB), lambda s: (0, cb(s))),
            pl.BlockSpec((4, CB), lambda s: (0, cb(s))),
            pl.BlockSpec((CB, S), lambda s: (cb(s), 0)),
            pl.BlockSpec((1, CB), lambda s: (0, cb(s))),
            full((2 * C, C)), full((C, 2 * C)),
            pl.BlockSpec((T, D), lambda s: (jnp.clip(s - NC, 0, NB - 1), 0)),
            full((1, D)), hbm, hbm, hbm, hbm, hbm,
        ],
        out_specs=pl.BlockSpec((T, D), lambda s: (jnp.clip(s - NC - 2, 0, NB - 1), 0)),
        out_shape=jax.ShapeDtypeStruct((S, D), BF),
        scratch_shapes=[
            vm((D, 6 * D), BF), vm((D, D), BF), vm((D, D), BF), vm((F, D), BF), vm((F, D), BF),
            pltpu.SemaphoreType.DMA((5,)),
            vm((S + PAD, CB), F32), vm((S, CB), F32),
            vm((3, P, C, CB), F32), vm((3, P, C, CB), F32), vm((P, 2, C, CB), BF),
            vm((NC, S, CB), F32), vm((8, 6 * D), F32),
            vm((S, D), F32), vm((S, D), F32), vm((S + 2 * PAD, D), F32),
        ],
        compiler_params=pltpu.CompilerParams(
            dimension_semantics=("arbitrary",), vmem_limit_bytes=100 * 1024 * 1024),
    )(A_k.reshape(S, D), A_v.reshape(S, D), A_shift_k.T, A_ssm_k, A_ssm_D.reshape(1, D),
      jnp.asarray(fwd), jnp.asarray(inv), A_q.reshape(S, D), c, w_mod, B_w1, B_w2, B_w3.T, B_w4)
    return out.reshape(1, S, D)
```
